```python
import os as _os
_os.environ.setdefault("JAX_PLATFORMS", "cpu")
import jax
import jax.numpy as jnp

def _softmax(x, axis=-1):
    return jax.nn.softmax(x, axis=axis)
def _gelu(x):
    return jax.nn.gelu(x, approximate=True)
def _silu(x):
    return jax.nn.silu(x)
def _sigmoid(x):
    return jax.nn.sigmoid(x)
def _layernorm(x, axis=-1, eps=1e-5):
    m = jnp.mean(x, axis=axis, keepdims=True)
    v = jnp.var(x, axis=axis, keepdims=True)
    return (x - m) / jnp.sqrt(v + eps)
def _scatter_add(tgt, idx, src, axis=0):
    return tgt.at[idx].add(src)
def _segment_sum(src, seg, n):
    return jax.ops.segment_sum(src, seg, n)
class _Rng:
    def __init__(self, key):
        self._k = key
    def _next(self):
        self._k, sub = jax.random.split(self._k)
        return sub
    def normal(self, shape):
        return jax.random.normal(self._next(), shape, dtype=jnp.bfloat16)
    def randint(self, lo, hi, shape):
        return jax.random.randint(self._next(), shape, lo, hi, dtype=jnp.int32)
    def uniform(self, shape, lo=0.0, hi=1.0):
        return jax.random.uniform(self._next(), shape, jnp.bfloat16, lo, hi)
    def permutation(self, n):
        return jax.random.permutation(self._next(), n)


kernel_name = 'sequential_preLN__compressed_kv_cla__dense_activation_mish__decode'

def setup_inputs():
    _rng = _Rng(jax.random.key(int.from_bytes(__import__("os").urandom(4), "little")))
    _w = (lambda a: (lambda t: t.astype(jnp.bfloat16) if jnp.issubdtype(t.dtype, jnp.floating) else t)(jnp.asarray(a)))
    def _A_setup():
        B, H, Sq, Sk, D, M = 2, 32, 1, 8192, 128, 512
        Dc = 4 * D
        return {
            "x": _w((lambda *s: _rng.normal(s) * 0.05)(B, Sq, M)),
            "c_kv": _w((lambda *s: _rng.normal(s) * 0.8)(B, Sk, Dc)),
            "w_q": _w((lambda *s: _rng.normal(s) * 0.8)(M, H, D) * (M ** -0.5)),
            "w_uk": _w((lambda *s: _rng.normal(s) * 0.8)(Dc, H, D) * (Dc ** -0.5)),
            "w_uv": _w((lambda *s: _rng.normal(s) * 0.8)(Dc, H, D) * (Dc ** -0.5)),
            "w_o": _w((lambda *s: _rng.normal(s) * 0.8)(H, D, M) * ((H * D) ** -0.5)),
        }
    _A_in = _A_setup()

    def _B_setup():
        B, S, D, F = 2, 1, 512, 1792
        return {
            "x": _w((lambda *s: _rng.normal(s) * 0.05)(B, S, D)),
            "w1": _w((lambda *s: _rng.normal(s) * 0.4)(D, F) * (D ** -0.5)),
            "b1": _w((lambda *s: _rng.normal(s) * 0.05)(F)),
            "w2": _w((lambda *s: _rng.normal(s) * 0.05)(F, D) * (F ** -0.5)),
        }
    _B_in = _B_setup()

    return {
        "A_x": _A_in["x"],
        "A_c_kv": _A_in["c_kv"],
        "A_w_q": _A_in["w_q"],
        "A_w_uk": _A_in["w_uk"],
        "A_w_uv": _A_in["w_uv"],
        "A_w_o": _A_in["w_o"],
        "B_x": _B_in["x"],
        "B_w1": _B_in["w1"],
        "B_b1": _B_in["b1"],
        "B_w2": _B_in["w2"],
    }

def reference(A_x, A_c_kv, A_w_q, A_w_uk, A_w_uv, A_w_o, B_x, B_w1, B_b1, B_w2):
    def _A_ref(x, c_kv, w_q, w_uk, w_uv, w_o):
        B, Sq, M = x.shape[0], x.shape[1], x.shape[2]
        Sk = c_kv.shape[1]
        H, D = w_q.shape[1], w_q.shape[2]
        q = jnp.einsum("bqm,mhd->bhqd", x, w_q)
        k = jnp.einsum("bkc,chd->bhkd", c_kv, w_uk)
        v = jnp.einsum("bkc,chd->bhkd", c_kv, w_uv)
        scores = jnp.einsum("bhqd,bhkd->bhqk", q, k) * (D ** -0.5)
        off = Sk - Sq
        qi = jnp.arange(Sq)[:, None]
        kj = jnp.arange(Sk)[None, :]
        cmask = kj <= (qi + off)
        scores = jnp.where(cmask[None, None], scores, -1e9)
        p = _softmax(scores, axis=-1)
        ctx = jnp.einsum("bhqk,bhkd->bhqd", p, v)
        return jnp.einsum("bhqd,hdm->bqm", ctx, w_o)

    def _B_ref(x, w1, b1, w2):
        h = jnp.einsum("bsd,df->bsf", x, w1) + b1
        sp = jnp.log1p(jnp.exp(-jnp.abs(h))) + jnp.where(h > 0, h, jnp.zeros_like(h))
        act = h * jnp.tanh(sp)
        return jnp.einsum("bsf,fd->bsd", act, w2)

    x = A_x
    h = x + _A_ref(_layernorm(x, axis=-1), A_c_kv, A_w_q, A_w_uk, A_w_uv, A_w_o)
    h2 = h + _B_ref(_layernorm(h, axis=-1), B_w1, B_b1, B_w2)
    return h2
```

```python
import jax
import jax.numpy as jnp
from jax import lax
from jax.experimental import pallas as pl
from jax.experimental.pallas import tpu as pltpu

NB = 2
H = 32
SK = 8192
D = 128
M = 512
DC = 512
F = 1792
RB = NB * H
LN_EPS = 1e-5
SCALE = D ** -0.5

TK = 1024
NT = SK // TK
NTILES = NB * NT
NBUF = 4
W = 2
W1_CH = ((0, 256), (256, 256))
W2_CH = ((0, 512), (512, 512), (1024, 512), (1536, 256))
M2 = M * H


def _ln(v):
    mu = jnp.mean(v, axis=-1, keepdims=True)
    cen = v - mu
    var = jnp.mean(cen * cen, axis=-1, keepdims=True)
    return cen / jnp.sqrt(var + LN_EPS)


def _nt(a, b):
    return lax.dot_general(a, b, (((1,), (1,)), ((), ())), preferred_element_type=jnp.float32)


def _nn(a, b):
    return jnp.dot(a, b, preferred_element_type=jnp.float32)


def _kernel(x_hbm, c_hbm, wq_hbm, wuk_hbm, wuv_hbm, wo_hbm, w1_hbm, b1_hbm, w2_hbm,
            o_ref,
            x_v, b1_v, wq_v, wuk_v, wuv_v, wo_v, w1_v, w2_v, cbuf, rtab,
            row_sc, qabs_sc, ctxa_sc, m_sc, l_sc, acc_sc,
            sem_small, sem_w, sem_c):
    bf16 = jnp.bfloat16
    f32 = jnp.float32

    nsem = [0]

    def item(src, dst):
        cp = pltpu.make_async_copy(src, dst, sem_w.at[nsem[0]])
        nsem[0] += 1
        return cp

    wq_items = [item(wq_hbm.at[pl.ds(4096 * i, 4096)], wq_v.at[pl.ds(4096 * i, 4096)]) for i in range(4)]
    wuk_items = [item(wuk_hbm.at[pl.ds(4096 * i, 4096)], wuk_v.at[pl.ds(4096 * i, 4096)]) for i in range(4)]
    wuv_items = [item(wuv_hbm.at[pl.ds(4096 * i, 4096)], wuv_v.at[pl.ds(4096 * i, 4096)]) for i in range(4)]
    wo_items = [item(wo_hbm.at[pl.ds(8 * i, 8)], wo_v.at[pl.ds(8 * i, 8)]) for i in range(4)]
    w1_items = [item(w1_hbm.at[pl.ds(s, n)], w1_v.at[pl.ds(s, n)]) for (s, n) in W1_CH]
    w2_items = [item(w2_hbm.at[pl.ds(s, n)], w2_v.at[pl.ds(s, n)]) for (s, n) in W2_CH]

    def c_copy(i, slot):
        b = i // NT
        t = i % NT
        return pltpu.make_async_copy(c_hbm.at[b, pl.ds(t * TK, TK)], cbuf.at[slot], sem_c.at[slot])

    pre_items = wq_items + wuk_items
    post_items = wuv_items + wo_items + w1_items + w2_items
    npre = len(pre_items)

    def start_global(g):
        if g < npre:
            pre_items[g].start()
        elif g < npre + NTILES:
            ti = g - npre
            c_copy(ti, ti % NBUF).start()
        elif g - npre - NTILES < len(post_items):
            post_items[g - npre - NTILES].start()

    x_cp = pltpu.make_async_copy(x_hbm, x_v, sem_small.at[0])
    b1_cp = pltpu.make_async_copy(b1_hbm, b1_v, sem_small.at[1])
    for g in range(W + 1):
        start_global(g)
    x_cp.start()
    b1_cp.start()

    kk = lax.broadcasted_iota(jnp.int32, (128, 128), 0)
    ll = lax.broadcasted_iota(jnp.int32, (128, 128), 1)
    for j in range(32):
        rtab[j] = jnp.where(kk == 4 * j + (ll >> 5), 1.0, 0.0).astype(bf16)
    rr = lax.broadcasted_iota(jnp.int32, (RB, 128), 0)
    lr = lax.broadcasted_iota(jnp.int32, (RB, 128), 1)
    dmask = (rr & 31) == (lr & 31)

    x_cp.wait()
    x2 = x_v[...].astype(f32)
    xn = _ln(x2)
    xrep = jnp.concatenate(
        [jnp.broadcast_to(xn[b:b + 1], (H, M)) for b in range(NB)], axis=0).astype(bf16)

    def head_contract(a_blk, w_v, i, acc):
        for j in range(32):
            e = _nn(a_blk, rtab[j])
            lhs = jnp.where(dmask, e, 0.0).astype(bf16)
            wt = w_v[pl.ds(4096 * i + 128 * j, 128), :]
            acc = acc + _nn(lhs, wt)
        return acc

    q_acc = jnp.zeros((RB, D), f32)
    for i in range(4):
        start_global(i + W + 1)
        wq_items[i].wait()
        q_acc = head_contract(xrep[:, 128 * i:128 * (i + 1)], wq_v, i, q_acc)
    q_bf = q_acc.astype(bf16)

    for i in range(4):
        start_global(4 + i + W + 1)
        wuk_items[i].wait()
        blk = jnp.zeros((RB, 128), f32)
        for j in range(32):
            wt = wuk_v[pl.ds(4096 * i + 128 * j, 128), :]
            z = _nt(q_bf, wt)
            zm = jnp.where(dmask, z * SCALE, 0.0).astype(bf16)
            blk = blk + _nt(zm, rtab[j])
        qabs_sc[:, 128 * i:128 * (i + 1)] = blk.astype(bf16)

    def body(it, carry):
        slot = it % NBUF
        b = it // NT
        t = it % NT

        @pl.when(it + W + 1 < NTILES)
        def _():
            nx = it + W + 1
            c_copy(nx, nx % NBUF).start()
        for k in range(W + 1):
            @pl.when(it == NTILES - (W + 1) + k)
            def _():
                post_items[k].start()

        c_copy(it, slot).wait()

        @pl.when(t == 0)
        def _():
            m_sc[...] = jnp.full(m_sc.shape, -jnp.inf, f32)
            l_sc[...] = jnp.zeros(l_sc.shape, f32)
            acc_sc[...] = jnp.zeros(acc_sc.shape, f32)

        c = cbuf[slot]
        qa = qabs_sc[pl.ds(pl.multiple_of(b * H, H), H), :]
        s = _nt(qa, c)
        m_old = m_sc[...]
        m_new = jnp.maximum(m_old, jnp.max(s, axis=1, keepdims=True))
        alpha = jnp.exp(m_old - m_new)
        p = jnp.exp(s - m_new)
        l_sc[...] = alpha * l_sc[...] + jnp.sum(p, axis=1, keepdims=True)
        acc_sc[...] = alpha * acc_sc[...] + _nn(p.astype(bf16), c)
        m_sc[...] = m_new

        @pl.when(t == NT - 1)
        def _():
            ctxa_sc[pl.ds(pl.multiple_of(b * H, H), H), :] = acc_sc[...] / l_sc[...]
        return carry

    lax.fori_loop(0, NTILES, body, 0)

    g0 = npre + NTILES
    a_bf = ctxa_sc[...].astype(bf16)
    ctx = jnp.zeros((RB, D), f32)
    for i in range(4):
        start_global(g0 + i + W + 1)
        wuv_items[i].wait()
        ctx = head_contract(a_bf[:, 128 * i:128 * (i + 1)], wuv_v, i, ctx)

    r8 = lax.broadcasted_iota(jnp.int32, (RB, 1024), 0) & 31
    l8 = lax.broadcasted_iota(jnp.int32, (RB, 1024), 1) >> 7
    ctx8 = jnp.concatenate([ctx] * 8, axis=1)
    a_acc = jnp.zeros((RB, M), f32)
    for i in range(4):
        start_global(g0 + 4 + i + W + 1)
        wo_items[i].wait()
        lbd = jnp.where(r8 == l8 + 8 * i, ctx8, 0.0).astype(bf16)
        a_acc = a_acc + _nn(lbd, wo_v[pl.ds(8 * i, 8)].reshape(1024, M))
    attn = jnp.concatenate(
        [jnp.sum(a_acc[b * H:(b + 1) * H], axis=0, keepdims=True) for b in range(NB)], axis=0)

    hres = x2 + attn
    hn = _ln(hres)
    row_sc[...] = jnp.zeros(row_sc.shape, f32)
    row_sc[0:NB, :] = hn
    hn16 = row_sc[...].astype(bf16)
    h1 = jnp.zeros((16, F), f32)
    for i, (s0, n0) in enumerate(W1_CH):
        start_global(g0 + 8 + i + W + 1)
        w1_items[i].wait()
        h1 = h1 + _nn(hn16[:, s0:s0 + n0], w1_v[pl.ds(s0, n0), :])
    b1_cp.wait()
    h1 = h1 + b1_v[...].astype(f32).reshape(1, F)
    sp = jnp.log1p(jnp.exp(-jnp.abs(h1))) + jnp.maximum(h1, 0.0)
    act = (h1 * jnp.tanh(sp)).astype(bf16)
    out = jnp.zeros((16, M), f32)
    for i, (s0, n0) in enumerate(W2_CH):
        start_global(g0 + 8 + len(W1_CH) + i + W + 1)
        w2_items[i].wait()
        out = out + _nn(act[:, s0:s0 + n0], w2_v[pl.ds(s0, n0), :])
    res = hres + out[0:NB, :]
    o_ref[...] = res.astype(o_ref.dtype)


@jax.jit
def pallas_sequential_preLN__compressed_kv_cla__dense_activation_mish__decode_kernel(
    A_x: jax.Array,
    A_c_kv: jax.Array,
    A_w_q: jax.Array,
    A_w_uk: jax.Array,
    A_w_uv: jax.Array,
    A_w_o: jax.Array,
    B_x: jax.Array,
    B_w1: jax.Array,
    B_b1: jax.Array,
    B_w2: jax.Array,
):
    bf16 = jnp.bfloat16
    f32 = jnp.float32
    n_w_items = 4 * 4 + len(W1_CH) + len(W2_CH)
    any_spec = pl.BlockSpec(memory_space=pl.ANY)
    out = pl.pallas_call(
        _kernel,
        out_shape=jax.ShapeDtypeStruct((NB, M), A_x.dtype),
        in_specs=[any_spec] * 9,
        out_specs=pl.BlockSpec(memory_space=pltpu.VMEM),
        scratch_shapes=[
            pltpu.VMEM((NB, M), bf16),
            pltpu.VMEM(B_b1.shape, bf16),
            pltpu.VMEM((M2, D), bf16),
            pltpu.VMEM((M2, D), bf16),
            pltpu.VMEM((M2, D), bf16),
            pltpu.VMEM(A_w_o.shape, bf16),
            pltpu.VMEM(B_w1.shape, bf16),
            pltpu.VMEM(B_w2.shape, bf16),
            pltpu.VMEM((NBUF, TK, DC), bf16),
            pltpu.VMEM((32, 128, 128), bf16),
            pltpu.VMEM((16, M), f32),
            pltpu.VMEM((RB, DC), bf16),
            pltpu.VMEM((RB, DC), f32),
            pltpu.VMEM((H, 1), f32),
            pltpu.VMEM((H, 1), f32),
            pltpu.VMEM((H, DC), f32),
            pltpu.SemaphoreType.DMA((2,)),
            pltpu.SemaphoreType.DMA((n_w_items,)),
            pltpu.SemaphoreType.DMA((NBUF,)),
        ],
        compiler_params=pltpu.CompilerParams(vmem_limit_bytes=64 * 1024 * 1024),
    )(A_x.reshape(NB, M), A_c_kv,
      A_w_q.reshape(M2, D), A_w_uk.reshape(M2, D), A_w_uv.reshape(M2, D),
      A_w_o, B_w1, B_b1, B_w2)
    return out.reshape(A_x.shape)
```
